```python
import os as _os
_os.environ.setdefault("JAX_PLATFORMS", "cpu")
import jax
import jax.numpy as jnp

def _softmax(x, axis=-1):
    return jax.nn.softmax(x, axis=axis)
def _gelu(x):
    return jax.nn.gelu(x, approximate=True)
def _silu(x):
    return jax.nn.silu(x)
def _sigmoid(x):
    return jax.nn.sigmoid(x)
def _layernorm(x, axis=-1, eps=1e-5):
    m = jnp.mean(x, axis=axis, keepdims=True)
    v = jnp.var(x, axis=axis, keepdims=True)
    return (x - m) / jnp.sqrt(v + eps)
def _scatter_add(tgt, idx, src, axis=0):
    return tgt.at[idx].add(src)
def _segment_sum(src, seg, n):
    return jax.ops.segment_sum(src, seg, n)
class _Rng:
    def __init__(self, key):
        self._k = key
    def _next(self):
        self._k, sub = jax.random.split(self._k)
        return sub
    def normal(self, shape):
        return jax.random.normal(self._next(), shape, dtype=jnp.bfloat16)
    def randint(self, lo, hi, shape):
        return jax.random.randint(self._next(), shape, lo, hi, dtype=jnp.int32)
    def uniform(self, shape, lo=0.0, hi=1.0):
        return jax.random.uniform(self._next(), shape, jnp.bfloat16, lo, hi)
    def permutation(self, n):
        return jax.random.permutation(self._next(), n)


kernel_name = 'gated_mix__mha_block__softmax_full_mha__prompt'

def setup_inputs():
    _rng = _Rng(jax.random.key(int.from_bytes(__import__("os").urandom(4), "little")))
    _w = (lambda a: (lambda t: t.astype(jnp.bfloat16) if jnp.issubdtype(t.dtype, jnp.floating) else t)(jnp.asarray(a)))
    def _A_setup():
        B, S, D, H = 1, 2048, 448, 16
        return {
            "x": _w((lambda *s: _rng.normal(s) * 0.05)(B, S, D)),
            "wqkv": _w((lambda *s: _rng.normal(s) * 0.4)(D, 3 * D)),
            "wo": _w((lambda *s: _rng.normal(s) * 0.05)(D, D)),
        }
    _A_in = _A_setup()

    def _B_setup():
        B, S, D = 1, 2048, 448
        return {
            "x": _w((lambda *s: _rng.normal(s) * 0.05)(B, S, D)),
            "wqkv": _w((lambda *s: _rng.normal(s) * 0.4)(D, 3 * D)),
            "wo": _w((lambda *s: _rng.normal(s) * 0.05)(D, D)),
        }
    _B_in = _B_setup()

    return {
        "A_x": _A_in["x"],
        "A_wqkv": _A_in["wqkv"],
        "A_wo": _A_in["wo"],
        "B_x": _B_in["x"],
        "B_wqkv": _B_in["wqkv"],
        "B_wo": _B_in["wo"],
        "gate_w": _w((lambda *s: _rng.normal(s) * 0.05)(448) * 16.0),
    }

def reference(A_x, A_wqkv, A_wo, B_x, B_wqkv, B_wo, gate_w):
    def _A_ref(x, wqkv, wo):
        B, S, D = x.shape
        H = 16
        Dh = D // H
        qkv = (lambda x, *d: x.transpose(*d))((x @ wqkv).reshape(B, S, 3, H, Dh), 2, 0, 3, 1, 4)
        q, k, v = qkv[0], qkv[1], qkv[2]
        scores = jnp.einsum("bhqd,bhkd->bhqk", q, k) * (Dh ** -0.5)
        p = _softmax(scores, axis=-1)
        o = jnp.einsum("bhqk,bhkd->bhqd", p, v)
        return (lambda x, *d: x.transpose(*d))(o, 0, 2, 1, 3).reshape(B, S, D) @ wo

    def _B_ref(x, wqkv, wo):
        B, S, D = x.shape
        H = 16; Dh = D // H
        qkv = (lambda x, *d: x.transpose(*d))((x @ wqkv).reshape(B, S, 3, H, Dh), 2, 0, 3, 1, 4)
        q, k, v = qkv[0], qkv[1], qkv[2]
        scale = Dh ** -0.5
        scores = jnp.einsum("bhqd,bhkd->bhqk", q, k) * scale
        p = _softmax(scores, axis=-1)
        o = jnp.einsum("bhqk,bhkd->bhqd", p, v)
        return (lambda x, *d: x.transpose(*d))(o, 0, 2, 1, 3).reshape(B, S, D) @ wo

    x = A_x
    g = _sigmoid((x * gate_w).sum(-1, keepdims=True))
    a = _A_ref(x, A_wqkv, A_wo)
    b = _B_ref(x, B_wqkv, B_wo)
    return g * a + (1 - g) * b
```

```python
import math

import jax
import jax.numpy as jnp
import jax.experimental.pallas as pl
import jax.experimental.pallas.tpu as pltpu

F32 = jnp.float32
BF16 = jnp.bfloat16

H = 16
DH = 28
DP = 32
BQ = 512
CK = 128
NT = (((1,), (1,)), ((), ()))
TN = (((0,), (0,)), ((), ()))


def _pad_heads_lanes(w, n):
    z = jnp.zeros((w.shape[0], DP - DH), w.dtype)
    parts = []
    for j in range(n):
        parts += [w[:, j * DH:(j + 1) * DH], z]
    return jnp.concatenate(parts, axis=1)


def _kernel(x_ref, wqa_ref, woa_ref, wqb_ref, wob_ref, gw_ref, out_ref,
            qt_ref, k_ref, vt_ref, s_ref, ot_ref, g_ref):
    S, D = x_ref.shape
    NQ = S // BQ
    NU = 2 * H * NQ
    GW = 4 * DP
    qscale = DH ** -0.5 * math.log2(math.e)

    row = jax.lax.broadcasted_iota(jnp.int32, (H * DP, BQ), 0)
    ones_row = (row % DP) == DH
    for b, w_ref in enumerate((wqa_ref, wqb_ref)):
        wp = _pad_heads_lanes(w_ref[...], 3 * H)
        wq_t = wp[:, 0:H * DP].T
        wk = wp[:, H * DP:2 * H * DP]
        wv_t = wp[:, 2 * H * DP:3 * H * DP].T
        for j in range(NQ):
            xs = x_ref[j * BQ:(j + 1) * BQ, :]
            q = jax.lax.dot_general(wq_t, xs, NT, preferred_element_type=F32)
            qt_ref[b * H * DP:(b + 1) * H * DP, j * BQ:(j + 1) * BQ] = (q * qscale).astype(BF16)
            v = jax.lax.dot_general(wv_t, xs, NT, preferred_element_type=F32)
            v = jnp.where(ones_row, 1.0, v)
            vt_ref[b * H * DP:(b + 1) * H * DP, j * BQ:(j + 1) * BQ] = v.astype(BF16)
            k = jnp.dot(xs, wk, preferred_element_type=F32).astype(BF16)
            for gi in range(4):
                k_ref[4 * b + gi, j * BQ:(j + 1) * BQ, :] = k[:, gi * GW:(gi + 1) * GW]
    gw = jnp.broadcast_to(gw_ref[...], (16, D))
    for j in range(NQ):
        xs = x_ref[j * BQ:(j + 1) * BQ, :]
        z = jax.lax.dot_general(gw, xs, NT, preferred_element_type=F32)[0:8]
        g = jax.nn.sigmoid(z)
        g_ref[0, :, j * BQ:(j + 1) * BQ] = g
        g_ref[1, :, j * BQ:(j + 1) * BQ] = 1.0 - g

    rows = jax.lax.broadcasted_iota(jnp.int32, (GW, BQ), 0)

    def get_q(u):
        hh = u // NQ
        g0 = pl.multiple_of((hh // 4) * GW, GW)
        q0 = pl.multiple_of((u % NQ) * BQ, BQ)
        qt = qt_ref[pl.ds(g0, GW), pl.ds(q0, BQ)]
        return hh // 4, jnp.where((rows // DP) == (hh % 4), qt, jnp.zeros_like(qt))

    def qk_chunk(g, qt, c, slot, m):
        s = jnp.dot(k_ref[g, c * CK:(c + 1) * CK, :], qt, preferred_element_type=F32)
        s_ref[slot, c * CK:(c + 1) * CK, :] = s
        return jnp.maximum(m, jnp.max(s.reshape(CK // 8, 8, BQ), axis=0))

    def m_init():
        return jnp.full((8, BQ), -jnp.inf, F32)

    def step(u, m_cur, slot, do_next):
        hh = u // NQ
        h0 = pl.multiple_of(hh * DP, DP)
        q0 = pl.multiple_of((u % NQ) * BQ, BQ)
        if do_next:
            gn, qtn = get_q(u + 1)
            m = m_init()
        acc = jnp.zeros((DP, BQ), F32)
        for c in range(S // CK):
            if do_next:
                m = qk_chunk(gn, qtn, c, 1 - slot, m)
            p = jnp.exp2(s_ref[slot, c * CK:(c + 1) * CK, :] - m_cur).astype(BF16)
            acc = acc + jnp.dot(vt_ref[pl.ds(h0, DP), c * CK:(c + 1) * CK], p,
                                preferred_element_type=F32)
        scale = g_ref[hh // H, 0:1, pl.ds(q0, BQ)] / acc[DH:DH + 1, :]
        ot_ref[pl.ds(h0, DP), pl.ds(q0, BQ)] = (acc * scale).astype(BF16)
        if do_next:
            return jnp.max(m, axis=0, keepdims=True)

    g, qt = get_q(0)
    m = m_init()
    for c in range(S // CK):
        m = qk_chunk(g, qt, c, 0, m)
    m0 = jnp.max(m, axis=0, keepdims=True)

    def body(i, m_cur):
        m1 = step(2 * i, m_cur, 0, True)
        return step(2 * i + 1, m1, 1, True)

    m_last = jax.lax.fori_loop(0, NU // 2 - 1, body, m0)
    m1 = step(NU - 2, m_last, 0, True)
    step(NU - 1, m1, 1, False)

    wo = []
    for w_ref in (woa_ref, wob_ref):
        w = w_ref[...]
        z = jnp.zeros((DP - DH, D), BF16)
        for h in range(H):
            wo += [w[h * DH:(h + 1) * DH, :], z]
    wo = jnp.concatenate(wo, axis=0)
    for j in range(NQ):
        o = jax.lax.dot_general(ot_ref[:, j * BQ:(j + 1) * BQ], wo, TN,
                                preferred_element_type=F32)
        out_ref[j * BQ:(j + 1) * BQ, :] = o.astype(out_ref.dtype)


@jax.jit
def pallas_gated_mix__mha_block__softmax_full_mha__prompt_kernel(
    A_x: jax.Array,
    A_wqkv: jax.Array,
    A_wo: jax.Array,
    B_x: jax.Array,
    B_wqkv: jax.Array,
    B_wo: jax.Array,
    gate_w: jax.Array,
):
    del B_x
    B, S, D = A_x.shape
    assert B == 1
    out = pl.pallas_call(
        _kernel,
        out_shape=jax.ShapeDtypeStruct((S, D), A_x.dtype),
        scratch_shapes=[
            pltpu.VMEM((2 * H * DP, S), BF16),
            pltpu.VMEM((8, S, 4 * DP), BF16),
            pltpu.VMEM((2 * H * DP, S), BF16),
            pltpu.VMEM((2, S, BQ), F32),
            pltpu.VMEM((2 * H * DP, S), BF16),
            pltpu.VMEM((2, 8, S), F32),
        ],
        compiler_params=pltpu.CompilerParams(vmem_limit_bytes=100 * 2**20),
    )(A_x.reshape(S, D), A_wqkv, A_wo, B_wqkv, B_wo, gate_w.reshape(1, D))
    return out.reshape(B, S, D)
```

```python
import functools
import math

import jax
import jax.numpy as jnp
import jax.experimental.pallas as pl
import jax.experimental.pallas.tpu as pltpu

F32 = jnp.float32
BF16 = jnp.bfloat16

H = 16
DH = 28
DP = 32
BQ = 512
CK = 128
CQ = 64
LEAD = 3
UB = 2
PB = 512
OB = 256
N_EARLY = 4


def _pad_heads_rows(y, pad):
    parts = []
    for h in range(H):
        parts += [y[h * DH:(h + 1) * DH, :], pad]
    return jnp.concatenate(parts, axis=0)


def _kernel(x_hbm, wqa_hbm, woa_hbm, wqb_hbm, wob_hbm, gw_hbm, out_hbm,
            qt_ref, k_ref, vt_ref, s_ref, ot_ref, g_ref, wt_ref, wot_ref,
            x_ref, wq_ref, wo_ref, gw_ref, out_ref, in_sems, out_sems):
    D, S = x_hbm.shape
    NQ = S // BQ
    NP = S // PB
    NO = S // OB
    GW = 4 * DP
    qscale = DH ** -0.5 * math.log2(math.e)

    def x_copy(j):
        return pltpu.make_async_copy(x_hbm.at[:, j * PB:(j + 1) * PB],
                                     x_ref.at[:, j * PB:(j + 1) * PB], in_sems.at[9 + j])

    w_pieces = ((0, 512), (512, 896), (896, 3 * D))

    def wq_copy(b, piece):
        lo, hi = w_pieces[piece]
        w_hbm = (wqa_hbm, wqb_hbm)[b]
        return pltpu.make_async_copy(w_hbm.at[:, lo:hi], wq_ref.at[b, :, lo:hi],
                                     in_sems.at[3 * b + piece])

    def wq_transpose(b, piece):
        lo, hi = w_pieces[piece]
        wt_ref[b, lo:hi, :] = wq_ref[b, :, lo:hi].T

    wo_copy = [pltpu.make_async_copy(w, wo_ref.at[b], in_sems.at[6 + b])
               for b, w in enumerate((woa_hbm, wob_hbm))]
    gw_copy = pltpu.make_async_copy(gw_hbm, gw_ref, in_sems.at[8])
    batches = (
        [wq_copy(0, 0), x_copy(0)],
        [wq_copy(0, 1), wq_copy(0, 2), gw_copy, x_copy(1)],
        [x_copy(j) for j in range(2, NP)] + [wq_copy(1, p) for p in range(3)] + wo_copy,
    )
    for batch in batches:
        for copy in batch:
            copy.start()

    def wait_batch(n):
        for copy in batches[n]:
            copy.wait()

    zpad = jnp.zeros((DP - DH, PB), F32)
    opad = (jax.lax.broadcasted_iota(jnp.int32, (DP - DH, PB), 0) == 0).astype(F32)

    def project(b, j, between=(None, None, None)):
        cols = slice(j * PB, (j + 1) * PB)
        r0, r1 = b * H * DP, (b + 1) * H * DP
        xs = x_ref[:, cols]
        if between[0]:
            between[0]()
        q = jnp.dot(wt_ref[b, 0:D, :], xs, preferred_element_type=F32)
        qt_ref[r0:r1, cols] = _pad_heads_rows(q * qscale, zpad).astype(BF16)
        if between[1]:
            between[1]()
        k = jnp.dot(wt_ref[b, D:2 * D, :], xs, preferred_element_type=F32)
        kn = _pad_heads_rows(k, zpad).astype(BF16).T
        for gi in range(4):
            k_ref[4 * b + gi, cols, :] = kn[:, gi * GW:(gi + 1) * GW]
        if between[2]:
            between[2]()
        v = jnp.dot(wt_ref[b, 2 * D:3 * D, :], xs, preferred_element_type=F32)
        vt_ref[r0:r1, cols] = _pad_heads_rows(v, opad).astype(BF16)

    def gate(j):
        cols = slice(j * PB, (j + 1) * PB)
        gw = jnp.broadcast_to(gw_ref[...].reshape(1, D), (16, D))
        z = jnp.dot(gw, x_ref[:, cols], preferred_element_type=F32)[0:8]
        g = jax.nn.sigmoid(z)
        g_ref[0, :, cols] = g
        g_ref[1, :, cols] = 1.0 - g

    def wo_transpose(b):
        wot_ref[:, b * D:(b + 1) * D] = wo_ref[b].T

    def second_batch():
        wait_batch(1)
        wq_transpose(0, 1)
        wq_transpose(0, 2)

    wait_batch(0)
    wq_transpose(0, 0)
    project(0, 0, (None, second_batch, None))
    gate(0)
    project(0, 1)
    gate(1)
    wait_batch(2)
    project(0, 2, [functools.partial(wq_transpose, 1, p) for p in range(3)])
    gate(2)
    for j in range(3, NP):
        project(0, j)
        gate(j)
    project(1, 0, (functools.partial(wo_transpose, 0), functools.partial(wo_transpose, 1), None))
    for j in range(1, NP):
        project(1, j)

    def out_copy(j):
        return pltpu.make_async_copy(out_ref.at[:, j * OB:(j + 1) * OB],
                                     out_hbm.at[:, j * OB:(j + 1) * OB], out_sems.at[j])

    def out_block(j):
        cols = slice(j * OB, (j + 1) * OB)
        o = jnp.dot(wot_ref[...], ot_ref[:, cols].astype(BF16), preferred_element_type=F32)
        out_ref[:, cols] = o.astype(out_ref.dtype)
        out_copy(j).start()

    NC = S // CK
    NCQ = S // CQ
    NG = 2 * H // 4

    def get_q(unit):
        g, qi, h = unit
        q0 = qi * BQ if isinstance(qi, int) else pl.multiple_of(qi * BQ, BQ)
        r0 = g * GW + h * DP
        r0 = r0 if isinstance(r0, int) else pl.multiple_of(r0, DP)
        parts = []
        if h > 0:
            parts.append(jnp.zeros((h * DP, BQ), BF16))
        parts.append(qt_ref[pl.ds(r0, DP), pl.ds(q0, BQ)])
        if h < 3:
            parts.append(jnp.zeros(((3 - h) * DP, BQ), BF16))
        return jnp.concatenate(parts, axis=0)

    def qk_chunk(g, qt, c, slot, m):
        s = jnp.dot(k_ref[g, c * CQ:(c + 1) * CQ, :], qt, preferred_element_type=F32)
        s_ref[slot, c * CQ:(c + 1) * CQ, :] = s
        s = jnp.max(s.reshape(CQ // 8, 8, BQ), axis=0)
        return s if m is None else jnp.maximum(m, s)

    def schedule(with_qk):
        if not with_qk:
            return [("pv", c) for c in range(NC)]
        order = [("qk", c) for c in range(LEAD)]
        n_pv = 0
        for c in range(LEAD, NCQ):
            target = ((c - LEAD + 1) * NC) // (NCQ - LEAD)
            while n_pv < target:
                order.append(("pv", n_pv))
                n_pv += 1
            order.append(("qk", c))
        return order

    def step(unit, slot, m_cur, nxt, fill=()):
        g, qi, h = unit
        dyn = not isinstance(g, int)
        q0 = qi * BQ if isinstance(qi, int) else pl.multiple_of(qi * BQ, BQ)
        h0 = g * GW + h * DP
        h0 = pl.multiple_of(h0, DP) if dyn else h0
        o0 = pl.multiple_of(g * 4 * DH, 8) if dyn else g * 4 * DH
        m = None
        if nxt is not None:
            qtn = get_q(nxt)
        acc = None
        for kind, c in schedule(nxt is not None):
            if kind == "qk":
                m = qk_chunk(nxt[0], qtn, c, 1 - slot, m)
                continue
            p = jnp.exp2(s_ref[slot, c * CK:(c + 1) * CK, :] - m_cur).astype(BF16)
            pv = jnp.dot(vt_ref[pl.ds(h0, DP), c * CK:(c + 1) * CK], p,
                         preferred_element_type=F32)
            acc = pv if acc is None else acc + pv
            if fill and c % (NC // len(fill)) == 0:
                fill[c // (NC // len(fill))]()
            if c == NC - 1:
                scale = g_ref[g // (NG // 2), 0:1, pl.ds(q0, BQ)] / acc[DH:DH + 1, :]
                o_blk = ot_ref.at[pl.ds(o0, 4 * DH), pl.ds(q0, BQ)]
                o_blk[h * DH:(h + 1) * DH, :] = (acc * scale)[0:DH, :]
        if nxt is not None:
            return jnp.max(m, axis=0, keepdims=True)

    qt = get_q((0, 0, 0))
    m = None
    for c in range(NCQ):
        m = qk_chunk(0, qt, c, 0, m)
    m_cur = jnp.max(m, axis=0, keepdims=True)

    NB = NG * NQ
    assert NQ & (NQ - 1) == 0
    q_bits = NQ.bit_length() - 1

    def first_unit(n):
        return (n >> q_bits, n & (NQ - 1), 0)

    def block(n, m_cur, last=False):
        g, qi, _ = first_unit(n)
        units = [(g, qi, h) for h in range(4)] + [None if last else first_unit(n + 1)]
        for h in range(4):
            fill = ()
            if last and h == 3:
                fill = [functools.partial(out_block, j) for j in range(N_EARLY)]
            m_cur = step(units[h], h % 2, m_cur, units[h + 1], fill)
        return m_cur

    def body(t, mm):
        for r in range(UB):
            mm = block(t * UB + r, mm)
        return mm

    n_loop = (NB - 1) // UB
    m_cur = jax.lax.fori_loop(0, n_loop, body, m_cur)
    for n in range(n_loop * UB, NB):
        m_cur = block(n, m_cur, last=(n == NB - 1))
    for j in range(N_EARLY, NO):
        out_block(j)
    for j in range(NO):
        out_copy(j).wait()

@jax.jit
def pallas_gated_mix__mha_block__softmax_full_mha__prompt_kernel(
    A_x: jax.Array,
    A_wqkv: jax.Array,
    A_wo: jax.Array,
    B_x: jax.Array,
    B_wqkv: jax.Array,
    B_wo: jax.Array,
    gate_w: jax.Array,
):
    del B_x
    B, S, D = A_x.shape
    assert B == 1
    out_t = pl.pallas_call(
        _kernel,
        out_shape=jax.ShapeDtypeStruct((D, S), A_x.dtype),
        in_specs=[pl.BlockSpec(memory_space=pl.ANY)] * 6,
        out_specs=pl.BlockSpec(memory_space=pl.ANY),
        scratch_shapes=[
            pltpu.VMEM((2 * H * DP, S), BF16),
            pltpu.VMEM((8, S, 4 * DP), BF16),
            pltpu.VMEM((2 * H * DP, S), BF16),
            pltpu.VMEM((2, S, BQ), F32),
            pltpu.VMEM((2 * H * DH, S), F32),
            pltpu.VMEM((2, 8, S), F32),
            pltpu.VMEM((2, 3 * D, D), BF16),
            pltpu.VMEM((D, 2 * D), BF16),
            pltpu.VMEM((D, S), BF16),
            pltpu.VMEM((2, D, 3 * D), BF16),
            pltpu.VMEM((2, D, D), BF16),
            pltpu.VMEM((D,), BF16),
            pltpu.VMEM((D, S), A_x.dtype),
            pltpu.SemaphoreType.DMA((9 + S // PB,)),
            pltpu.SemaphoreType.DMA((S // OB,)),
        ],
        compiler_params=pltpu.CompilerParams(vmem_limit_bytes=100 * 2**20),
    )(A_x.reshape(S, D).T, A_wqkv, A_wo, B_wqkv, B_wo, gate_w)
    return out_t.T.reshape(B, S, D)
```

```python
import functools
import math

import jax
import jax.numpy as jnp
import jax.experimental.pallas as pl
import jax.experimental.pallas.tpu as pltpu

F32 = jnp.float32
BF16 = jnp.bfloat16
U32 = jnp.uint32

H = 16
DH = 28
DP = 32
BQ = 512
CK = 128
CQ = 64
LEAD = 3
NW = 2
UB = 2
PB = 512
OB = 256
N_EARLY = 4


def _pack(y):
    return pltpu.bitcast(y.astype(BF16), U32)


def _unpack(w):
    return pltpu.bitcast(w, BF16)


def _pad_heads_rows(y, pad):
    parts = []
    for h in range(H):
        parts += [y[h * DH:(h + 1) * DH, :], pad]
    return jnp.concatenate(parts, axis=0)


def _kernel(x_hbm, wqa_hbm, woa_hbm, wqb_hbm, wob_hbm, gw_hbm, out_hbm,
            qt_ref, k_ref, vt_ref, s_ref, ot_ref, g_ref, wt_ref, wot_ref,
            x_ref, wq_ref, wo_ref, gw_ref, out_ref, in_sems, out_sems):
    D, S = x_hbm.shape
    NQ = S // BQ
    NP = S // PB
    NO = S // OB
    GW = 4 * DP
    qscale = DH ** -0.5 * math.log2(math.e)

    def x_copy(j):
        return pltpu.make_async_copy(x_hbm.at[:, j * PB:(j + 1) * PB],
                                     x_ref.at[:, j * PB:(j + 1) * PB], in_sems.at[9 + j])

    w_pieces = ((0, 512), (512, 896), (896, 3 * D))

    def wq_copy(b, piece):
        lo, hi = w_pieces[piece]
        w_hbm = (wqa_hbm, wqb_hbm)[b]
        return pltpu.make_async_copy(w_hbm.at[:, lo:hi], wq_ref.at[b, :, lo:hi],
                                     in_sems.at[3 * b + piece])

    def wq_transpose(b, piece):
        lo, hi = w_pieces[piece]
        wt_ref[b, lo // 2:hi // 2, :] = _pack(wq_ref[b, :, lo:hi].T)

    wo_copy = [pltpu.make_async_copy(w, wo_ref.at[b], in_sems.at[6 + b])
               for b, w in enumerate((woa_hbm, wob_hbm))]
    gw_copy = pltpu.make_async_copy(gw_hbm, gw_ref, in_sems.at[8])
    batches = (
        [wq_copy(0, 0), x_copy(0)],
        [wq_copy(0, 1), wq_copy(0, 2), gw_copy],
        [x_copy(j) for j in range(1, NP)],
        [wq_copy(1, p) for p in range(3)] + wo_copy,
    )
    for batch in batches:
        for copy in batch:
            copy.start()

    def wait_batch(n):
        for copy in batches[n]:
            copy.wait()

    zpad = jnp.zeros((DP - DH, PB), F32)
    opad = (jax.lax.broadcasted_iota(jnp.int32, (DP - DH, PB), 0) == 0).astype(F32)

    def project(b, j, between=(None, None, None)):
        cols = slice(j * PB, (j + 1) * PB)
        r0, r1 = b * H * DP, (b + 1) * H * DP
        xs = x_ref[:, cols]
        if between[0]:
            between[0]()
        q = jnp.dot(_unpack(wt_ref[b, 0:D // 2, :]), xs, preferred_element_type=F32)
        qt_ref[r0 // 2:r1 // 2, cols] = _pack(_pad_heads_rows(q * qscale, zpad))
        if between[1]:
            between[1]()
        k = jnp.dot(_unpack(wt_ref[b, D // 2:D, :]), xs, preferred_element_type=F32)
        kn = _pad_heads_rows(k, zpad).astype(BF16).T
        for gi in range(4):
            k_ref[4 * b + gi, j * PB // 2:(j + 1) * PB // 2, :] = pltpu.bitcast(
                kn[:, gi * GW:(gi + 1) * GW], U32)
        if between[2]:
            between[2]()
        v = jnp.dot(_unpack(wt_ref[b, D:3 * D // 2, :]), xs, preferred_element_type=F32)
        vt_ref[r0 // 2:r1 // 2, cols] = _pack(_pad_heads_rows(v, opad))

    def gate(j):
        cols = slice(j * PB, (j + 1) * PB)
        gw = jnp.broadcast_to(gw_ref[...].reshape(1, D), (16, D))
        z = jnp.dot(gw, x_ref[:, cols], preferred_element_type=F32)[0:8]
        g = jax.nn.sigmoid(z)
        g_ref[0, :, cols] = g
        g_ref[1, :, cols] = 1.0 - g

    def wo_transpose(b):
        wot_ref[:, b * D:(b + 1) * D] = _pack(wo_ref[b].T)

    def second_batch():
        wait_batch(1)
        wq_transpose(0, 1)
        wq_transpose(0, 2)

    wait_batch(0)
    wq_transpose(0, 0)
    project(0, 0, (None, second_batch, None))
    gate(0)
    wait_batch(2)
    project(0, 1)
    gate(1)
    wait_batch(3)
    project(0, 2, [functools.partial(wq_transpose, 1, p) for p in range(3)])
    gate(2)
    for j in range(3, NP):
        project(0, j)
        gate(j)
    project(1, 0, (functools.partial(wo_transpose, 0), functools.partial(wo_transpose, 1), None))
    for j in range(1, NP):
        project(1, j)

    def out_copy(j):
        return pltpu.make_async_copy(out_ref.at[:, j * OB:(j + 1) * OB],
                                     out_hbm.at[:, j * OB:(j + 1) * OB], out_sems.at[j])

    def out_block(j):
        cols = slice(j * OB, (j + 1) * OB)
        o = jnp.dot(_unpack(wot_ref[...]), ot_ref[:, cols].astype(BF16), preferred_element_type=F32)
        out_ref[:, cols] = o.astype(out_ref.dtype)
        out_copy(j).start()

    NC = S // CK
    NCQ = S // CQ
    NG = 2 * H // 4

    def get_q(unit):
        g, qi, h = unit
        q0 = qi * BQ if isinstance(qi, int) else pl.multiple_of(qi * BQ, BQ)
        r0 = g * (GW // 2) + h * (DP // 2)
        r0 = r0 if isinstance(r0, int) else pl.multiple_of(r0, DP // 2)
        parts = []
        if h > 0:
            parts.append(jnp.zeros((h * DP, BQ), BF16))
        parts.append(_unpack(qt_ref[pl.ds(r0, DP // 2), pl.ds(q0, BQ)]))
        if h < 3:
            parts.append(jnp.zeros(((3 - h) * DP, BQ), BF16))
        return jnp.concatenate(parts, axis=0)

    def qk_chunk(g, qt, c, slot, m):
        k = _unpack(k_ref[g, c * CQ // 2:(c + 1) * CQ // 2, :])
        s = jnp.dot(k, qt, preferred_element_type=F32)
        s_ref[slot, c * CQ:(c + 1) * CQ, :] = s
        s = jnp.max(s.reshape(CQ // 8, 8, BQ), axis=0)
        return s if m is None else jnp.maximum(m, s)

    def schedule(with_qk):
        if not with_qk:
            return [("pv", c) for c in range(NC)]
        order = [("qk", c) for c in range(LEAD)]
        n_pv = 0
        for c in range(LEAD, NCQ):
            target = ((c - LEAD + 1) * NC) // (NCQ - LEAD)
            while n_pv < target:
                order.append(("pv", n_pv))
                n_pv += 1
            order.append(("qk", c))
        return order

    def step(unit, slot, m_cur, nxt, fill=()):
        g, qi, h = unit
        dyn = not isinstance(g, int)
        q0 = qi * BQ if isinstance(qi, int) else pl.multiple_of(qi * BQ, BQ)
        h0 = g * (GW // 2) + h * (DP // 2)
        h0 = pl.multiple_of(h0, DP // 2) if dyn else h0
        o0 = pl.multiple_of(g * 4 * DH, 8) if dyn else g * 4 * DH
        m = None
        if nxt is not None:
            qtn = get_q(nxt)
        acc = [None] * NW
        for kind, c in schedule(nxt is not None):
            if kind == "qk":
                m = qk_chunk(nxt[0], qtn, c, 1 - slot, m)
                continue
            vt = _unpack(vt_ref[pl.ds(h0, DP // 2), c * CK:(c + 1) * CK])
            for w in range(NW):
                lanes = slice(w * BQ // NW, (w + 1) * BQ // NW)
                s = s_ref[slot, c * CK:(c + 1) * CK, lanes]
                p = jnp.exp2(s - m_cur[:, lanes]).astype(BF16)
                pv = jnp.dot(vt, p, preferred_element_type=F32)
                acc[w] = pv if c == 0 else acc[w] + pv
            if fill and c % (NC // len(fill)) == 0:
                fill[c // (NC // len(fill))]()
            if c == NC - 1:
                o_blk = ot_ref.at[pl.ds(o0, 4 * DH), pl.ds(q0, BQ)]
                gate_row = g_ref[g // (NG // 2), 0:1, pl.ds(q0, BQ)]
                for w in range(NW):
                    lanes = slice(w * BQ // NW, (w + 1) * BQ // NW)
                    scale = gate_row[:, lanes] / acc[w][DH:DH + 1, :]
                    o_blk[h * DH:(h + 1) * DH, lanes] = (acc[w] * scale)[0:DH, :]
        if nxt is not None:
            return jnp.max(m, axis=0, keepdims=True)

    qt = get_q((0, 0, 0))
    m = None
    for c in range(NCQ):
        m = qk_chunk(0, qt, c, 0, m)
    m_cur = jnp.max(m, axis=0, keepdims=True)

    NB = NG * NQ
    assert NQ & (NQ - 1) == 0
    assert N_EARLY * OB <= (NQ - 1) * BQ
    q_bits = NQ.bit_length() - 1

    def first_unit(n):
        return (n >> q_bits, n & (NQ - 1), 0)

    def block(n, m_cur, last=False):
        g, qi, _ = first_unit(n)
        units = [(g, qi, h) for h in range(4)] + [None if last else first_unit(n + 1)]
        for h in range(4):
            fill = ()
            if last and h == 3:
                fill = [functools.partial(out_block, j) for j in range(N_EARLY)]
            m_cur = step(units[h], h % 2, m_cur, units[h + 1], fill)
        return m_cur

    def body(t, mm):
        for r in range(UB):
            mm = block(t * UB + r, mm)
        return mm

    n_loop = (NB - 1) // UB
    m_cur = jax.lax.fori_loop(0, n_loop, body, m_cur)
    for n in range(n_loop * UB, NB):
        m_cur = block(n, m_cur, last=(n == NB - 1))
    for j in range(N_EARLY, NO):
        out_block(j)
    for j in range(NO):
        out_copy(j).wait()


@jax.jit
def pallas_gated_mix__mha_block__softmax_full_mha__prompt_kernel(
    A_x: jax.Array,
    A_wqkv: jax.Array,
    A_wo: jax.Array,
    B_x: jax.Array,
    B_wqkv: jax.Array,
    B_wo: jax.Array,
    gate_w: jax.Array,
):
    del B_x
    B, S, D = A_x.shape
    assert B == 1
    out_t = pl.pallas_call(
        _kernel,
        out_shape=jax.ShapeDtypeStruct((D, S), A_x.dtype),
        in_specs=[pl.BlockSpec(memory_space=pl.ANY)] * 6,
        out_specs=pl.BlockSpec(memory_space=pl.ANY),
        scratch_shapes=[
            pltpu.VMEM((H * DP, S), U32),
            pltpu.VMEM((8, S // 2, 4 * DP), U32),
            pltpu.VMEM((H * DP, S), U32),
            pltpu.VMEM((2, S, BQ), F32),
            pltpu.VMEM((2 * H * DH, S), F32),
            pltpu.VMEM((2, 8, S), F32),
            pltpu.VMEM((2, 3 * D // 2, D), U32),
            pltpu.VMEM((D // 2, 2 * D), U32),
            pltpu.VMEM((D, S), BF16),
            pltpu.VMEM((2, D, 3 * D), BF16),
            pltpu.VMEM((2, D, D), BF16),
            pltpu.VMEM((D,), BF16),
            pltpu.VMEM((D, S), A_x.dtype),
            pltpu.SemaphoreType.DMA((9 + S // PB,)),
            pltpu.SemaphoreType.DMA((S // OB,)),
        ],
        compiler_params=pltpu.CompilerParams(vmem_limit_bytes=100 * 2**20),
    )(A_x.reshape(S, D).T, A_wqkv, A_wo, B_wqkv, B_wo, gate_w)
    return out_t.T.reshape(B, S, D)
```
